```python
import os as _os
_os.environ.setdefault("JAX_PLATFORMS", "cpu")
import jax
import jax.numpy as jnp

def _softmax(x, axis=-1):
    return jax.nn.softmax(x, axis=axis)
def _gelu(x):
    return jax.nn.gelu(x, approximate=True)
def _silu(x):
    return jax.nn.silu(x)
def _sigmoid(x):
    return jax.nn.sigmoid(x)
def _layernorm(x, axis=-1, eps=1e-5):
    m = jnp.mean(x, axis=axis, keepdims=True)
    v = jnp.var(x, axis=axis, keepdims=True)
    return (x - m) / jnp.sqrt(v + eps)
def _scatter_add(tgt, idx, src, axis=0):
    return tgt.at[idx].add(src)
def _segment_sum(src, seg, n):
    return jax.ops.segment_sum(src, seg, n)
class _Rng:
    def __init__(self, key):
        self._k = key
    def _next(self):
        self._k, sub = jax.random.split(self._k)
        return sub
    def normal(self, shape):
        return jax.random.normal(self._next(), shape, dtype=jnp.bfloat16)
    def randint(self, lo, hi, shape):
        return jax.random.randint(self._next(), shape, lo, hi, dtype=jnp.int32)
    def uniform(self, shape, lo=0.0, hi=1.0):
        return jax.random.uniform(self._next(), shape, jnp.bfloat16, lo, hi)
    def permutation(self, n):
        return jax.random.permutation(self._next(), n)


kernel_name = 'gated_mix__mha_block__softmax_full_mha__prompt'

def setup_inputs():
    _rng = _Rng(jax.random.key(int.from_bytes(__import__("os").urandom(4), "little")))
    _w = (lambda a: (lambda t: t.astype(jnp.bfloat16) if jnp.issubdtype(t.dtype, jnp.floating) else t)(jnp.asarray(a)))
    def _A_setup():
        B, S, D, H = 1, 2048, 448, 16
        return {
            "x": _w((lambda *s: _rng.normal(s) * 0.05)(B, S, D)),
            "wqkv": _w((lambda *s: _rng.normal(s) * 0.4)(D, 3 * D)),
            "wo": _w((lambda *s: _rng.normal(s) * 0.05)(D, D)),
        }
    _A_in = _A_setup()

    def _B_setup():
        B, S, D = 1, 2048, 448
        return {
            "x": _w((lambda *s: _rng.normal(s) * 0.05)(B, S, D)),
            "wqkv": _w((lambda *s: _rng.normal(s) * 0.4)(D, 3 * D)),
            "wo": _w((lambda *s: _rng.normal(s) * 0.05)(D, D)),
        }
    _B_in = _B_setup()

    return {
        "A_x": _A_in["x"],
        "A_wqkv": _A_in["wqkv"],
        "A_wo": _A_in["wo"],
        "B_x": _B_in["x"],
        "B_wqkv": _B_in["wqkv"],
        "B_wo": _B_in["wo"],
        "gate_w": _w((lambda *s: _rng.normal(s) * 0.05)(448) * 16.0),
    }

def reference(A_x, A_wqkv, A_wo, B_x, B_wqkv, B_wo, gate_w):
    def _A_ref(x, wqkv, wo):
        B, S, D = x.shape
        H = 16
        Dh = D // H
        qkv = (lambda x, *d: x.transpose(*d))((x @ wqkv).reshape(B, S, 3, H, Dh), 2, 0, 3, 1, 4)
        q, k, v = qkv[0], qkv[1], qkv[2]
        scores = jnp.einsum("bhqd,bhkd->bhqk", q, k) * (Dh ** -0.5)
        p = _softmax(scores, axis=-1)
        o = jnp.einsum("bhqk,bhkd->bhqd", p, v)
        return (lambda x, *d: x.transpose(*d))(o, 0, 2, 1, 3).reshape(B, S, D) @ wo

    def _B_ref(x, wqkv, wo):
        B, S, D = x.shape
        H = 16; Dh = D // H
        qkv = (lambda x, *d: x.transpose(*d))((x @ wqkv).reshape(B, S, 3, H, Dh), 2, 0, 3, 1, 4)
        q, k, v = qkv[0], qkv[1], qkv[2]
        scale = Dh ** -0.5
        scores = jnp.einsum("bhqd,bhkd->bhqk", q, k) * scale
        p = _softmax(scores, axis=-1)
        o = jnp.einsum("bhqk,bhkd->bhqd", p, v)
        return (lambda x, *d: x.transpose(*d))(o, 0, 2, 1, 3).reshape(B, S, D) @ wo

    x = A_x
    g = _sigmoid((x * gate_w).sum(-1, keepdims=True))
    a = _A_ref(x, A_wqkv, A_wo)
    b = _B_ref(x, B_wqkv, B_wo)
    return g * a + (1 - g) * b
```

```python
import functools
import math

import jax
import jax.numpy as jnp
import jax.experimental.pallas as pl
import jax.experimental.pallas.tpu as pltpu

S = 2048
D = 448
H = 16
DH = 28
HP = 32
DP = H * HP
NH = 2 * H
NG = NH // 4
BQ = 256
NQ = S // BQ
QSCALE = (DH ** -0.5) * math.log2(math.e)


def _kernel(x_ref, wqT_ref, wk_ref, wvT_ref, wo_ref, gw_ref, o_ref,
            k_scr, qT_scr, vT_scr, g_scr, oT_scr):
    step = pl.program_id(0)

    @pl.when(step == 0)
    def _():
        x = x_ref[...]
        for mod in range(2):
            kf = jnp.dot(x, wk_ref[mod], preferred_element_type=jnp.float32)
            for j in range(4):
                k_scr[4 * mod + j] = kf[:, 128 * j:128 * (j + 1)].astype(jnp.bfloat16)
            qf = jax.lax.dot_general(wqT_ref[mod], x, (((1,), (1,)), ((), ())),
                                     preferred_element_type=jnp.float32)
            qf = (qf * QSCALE).astype(jnp.bfloat16)
            for j in range(4):
                qT_scr[4 * mod + j] = qf[128 * j:128 * (j + 1), :]
            vf = jax.lax.dot_general(wvT_ref[mod], x, (((1,), (1,)), ((), ())),
                                     preferred_element_type=jnp.float32)
            rows = jax.lax.broadcasted_iota(jnp.int32, vf.shape, 0)
            vf = jnp.where((rows & (HP - 1)) == DH, 1.0, vf).astype(jnp.bfloat16)
            for j in range(H):
                vT_scr[H * mod + j] = vf[HP * j:HP * (j + 1), :]
        gw = jnp.broadcast_to(gw_ref[...], (8, D))
        gl = jax.lax.dot_general(gw, x, (((1,), (1,)), ((), ())),
                                 preferred_element_type=jnp.float32)
        g_scr[...] = jax.nn.sigmoid(gl)

    q0 = pl.multiple_of(step * BQ, BQ)
    g = g_scr[0:1, pl.ds(q0, BQ)]

    def head_body(h, carry):
        grp = h // 4
        sub = h % 4
        qT = qT_scr[grp, :, pl.ds(q0, BQ)]
        rows = jax.lax.broadcasted_iota(jnp.int32, (128, BQ), 0)
        qm = jnp.where((rows // HP) == sub, qT, jnp.zeros_like(qT))
        sT = jnp.dot(k_scr[grp], qm, preferred_element_type=jnp.float32)
        m = jnp.max(sT, axis=0, keepdims=True)
        p = jnp.exp2(sT - m).astype(jnp.bfloat16)
        oT = jnp.dot(vT_scr[h], p, preferred_element_type=jnp.float32)
        l = oT[DH:DH + 1, :]
        gate = jnp.where(h < H, g, 1.0 - g)
        oT_scr[h] = (oT * (gate / l)).astype(jnp.bfloat16)
        return carry

    jax.lax.fori_loop(0, NH, head_body, 0)
    oT = oT_scr[...].reshape(NH * HP, BQ)
    out = jax.lax.dot_general(oT, wo_ref[...], (((0,), (0,)), ((), ())),
                              preferred_element_type=jnp.float32)
    o_ref[...] = out.astype(o_ref.dtype)


def _prep_qkv(w):
    w = w.reshape(D, 3, H, DH)
    w = jnp.pad(w, ((0, 0), (0, 0), (0, 0), (0, HP - DH))).reshape(D, 3, DP)
    return w[:, 0].T, w[:, 1], w[:, 2].T


def _prep_o(w):
    w = w.reshape(H, DH, D)
    return jnp.pad(w, ((0, 0), (0, HP - DH), (0, 0))).reshape(DP, D)


@jax.jit
def pallas_gated_mix__mha_block__softmax_full_mha__prompt_kernel(
    A_x: jax.Array,
    A_wqkv: jax.Array,
    A_wo: jax.Array,
    B_x: jax.Array,
    B_wqkv: jax.Array,
    B_wo: jax.Array,
    gate_w: jax.Array,
):
    x = A_x.reshape(S, D)
    aq, ak, av = _prep_qkv(A_wqkv)
    bq, bk, bv = _prep_qkv(B_wqkv)
    wqT = jnp.stack([aq, bq])
    wk = jnp.stack([ak, bk])
    wvT = jnp.stack([av, bv])
    wo = jnp.concatenate([_prep_o(A_wo), _prep_o(B_wo)], axis=0)
    gw = gate_w.reshape(1, D)

    full = lambda shape: pl.BlockSpec(shape, lambda i: (0,) * len(shape))
    out = pl.pallas_call(
        _kernel,
        grid=(NQ,),
        in_specs=[full((S, D)), full((2, DP, D)), full((2, D, DP)), full((2, DP, D)),
                  full((2 * DP, D)), full((1, D))],
        out_specs=pl.BlockSpec((BQ, D), lambda i: (i, 0)),
        out_shape=jax.ShapeDtypeStruct((S, D), jnp.bfloat16),
        scratch_shapes=[
            pltpu.VMEM((NG, S, 128), jnp.bfloat16),
            pltpu.VMEM((NG, 128, S), jnp.bfloat16),
            pltpu.VMEM((NH, HP, S), jnp.bfloat16),
            pltpu.VMEM((8, S), jnp.float32),
            pltpu.VMEM((NH, HP, BQ), jnp.bfloat16),
        ],
        compiler_params=pltpu.CompilerParams(
            dimension_semantics=("arbitrary",),
            vmem_limit_bytes=100 * 1024 * 1024),
    )(x, wqT, wk, wvT, wo, gw)
    return out.reshape(1, S, D)
```

```python
import functools
import math

import jax
import jax.numpy as jnp
import jax.experimental.pallas as pl
import jax.experimental.pallas.tpu as pltpu

S = 2048
D = 448
H = 16
DH = 28
HP = 32
DP = H * HP
NH = 2 * H
NG = NH // 4
BQ = 512
NQ = S // BQ
CK = 256
NC = S // CK
QSCALE = (DH ** -0.5) * math.log2(math.e)


def _kernel(xT_ref, wa_ref, wb_ref, woa_ref, wob_ref, gw_ref, o_ref,
            k_scr, qT_scr, vT_scr, woT_scr, g_scr, oT_scr, sa_scr, sb_scr, m_scr):
    step = pl.program_id(0)

    def qmask(hn, qn):
        grp = hn // 4
        sub = hn % 4
        qT = qT_scr[grp, :, pl.ds(pl.multiple_of(qn * BQ, BQ), BQ)]
        rows = jax.lax.broadcasted_iota(jnp.int32, (128, BQ), 0)
        return jnp.where((rows // HP) == sub, qT, jnp.zeros_like(qT))

    def qk_chunk(hn, qm, c, s_nxt, m_part):
        s = jnp.dot(k_scr[hn // 4, c * CK:(c + 1) * CK, :], qm,
                    preferred_element_type=jnp.float32)
        s_nxt[c * CK:(c + 1) * CK, :] = s
        mx = jnp.max(s.reshape(CK // 8, 8, BQ), axis=0)
        return mx if m_part is None else jnp.maximum(m_part, mx)

    @pl.when(step == 0)
    def _():
        xT = xT_ref[...]
        x = xT.T
        tn = (((0,), (0,)), ((), ()))
        for mod, (w_ref, wo_ref) in enumerate(((wa_ref, woa_ref), (wb_ref, wob_ref))):
            parts = []
            for h in range(H):
                parts.append(w_ref[:, D + DH * h:D + DH * (h + 1)])
                parts.append(jnp.zeros((D, HP - DH), jnp.bfloat16))
            wk = jnp.concatenate(parts, axis=1)
            kf = jnp.dot(x, wk, preferred_element_type=jnp.float32)
            for j in range(4):
                k_scr[4 * mod + j] = kf[:, 128 * j:128 * (j + 1)].astype(jnp.bfloat16)
            qf = jax.lax.dot_general(w_ref[:, 0:D], xT, tn, preferred_element_type=jnp.float32)
            qf = qf * QSCALE
            zpad = jnp.zeros((HP - DH, S), jnp.float32)
            for h in range(H):
                blk = jnp.concatenate([qf[DH * h:DH * (h + 1), :], zpad], axis=0)
                qT_scr[4 * mod + h // 4, HP * (h % 4):HP * (h % 4 + 1), :] = blk.astype(jnp.bfloat16)
            vf = jax.lax.dot_general(w_ref[:, 2 * D:3 * D], xT, tn, preferred_element_type=jnp.float32)
            rows = jax.lax.broadcasted_iota(jnp.int32, (HP - DH, S), 0)
            opad = jnp.where(rows == 0, 1.0, 0.0).astype(jnp.float32)
            for h in range(H):
                blk = jnp.concatenate([vf[DH * h:DH * (h + 1), :], opad], axis=0)
                vT_scr[H * mod + h] = blk.astype(jnp.bfloat16)
            parts = []
            for h in range(H):
                parts.append(wo_ref[DH * h:DH * (h + 1), :])
                parts.append(jnp.zeros((HP - DH, D), jnp.bfloat16))
            wo_pad = jnp.concatenate(parts, axis=0)
            woT_scr[:, DP * mod:DP * (mod + 1)] = wo_pad.T
        gw = jnp.broadcast_to(gw_ref[...], (8, D))
        gl = jnp.dot(gw, xT, preferred_element_type=jnp.float32)
        g_scr[...] = jax.nn.sigmoid(gl)

    @pl.when(step == 0)
    def _():
        qm0 = qmask(0, 0)
        mp = None
        for c in range(NC):
            mp = qk_chunk(0, qm0, c, sa_scr, mp)
        m_scr[...] = jnp.broadcast_to(jnp.max(mp, axis=0, keepdims=True), (8, BQ))

    q0 = pl.multiple_of(step * BQ, BQ)

    def stage(h, s_cur, s_nxt):
        last = h == NH - 1
        hn = jnp.where(last, 0, h + 1)
        qn = jnp.where(last, jnp.minimum(step + 1, NQ - 1), step)
        m_cur = m_scr[0:1, :]
        qm = qmask(hn, qn)
        m_part = None
        acc = None
        for c in range(NC):
            m_part = qk_chunk(hn, qm, c, s_nxt, m_part)
            p = jnp.exp2(s_cur[c * CK:(c + 1) * CK, :] - m_cur).astype(jnp.bfloat16)
            d = jnp.dot(vT_scr[h, :, c * CK:(c + 1) * CK], p,
                        preferred_element_type=jnp.float32)
            acc = d if acc is None else acc + d
        l = acc[DH:DH + 1, :]
        g = g_scr[0:1, pl.ds(q0, BQ)]
        gate = jnp.where(h < H, g, 1.0 - g)
        oT_scr[h] = (acc * (gate / l)).astype(jnp.bfloat16)
        m_scr[...] = jnp.broadcast_to(jnp.max(m_part, axis=0, keepdims=True), (8, BQ))

    def body(h, carry):
        @pl.when(h % 2 == 0)
        def _():
            stage(h, sa_scr, sb_scr)

        @pl.when(h % 2 == 1)
        def _():
            stage(h, sb_scr, sa_scr)
        return carry

    jax.lax.fori_loop(0, NH, body, 0)
    oT = oT_scr[...].reshape(NH * HP, BQ)
    outT = jnp.dot(woT_scr[...], oT, preferred_element_type=jnp.float32)
    o_ref[...] = outT.astype(o_ref.dtype)


@jax.jit
def pallas_gated_mix__mha_block__softmax_full_mha__prompt_kernel(
    A_x: jax.Array,
    A_wqkv: jax.Array,
    A_wo: jax.Array,
    B_x: jax.Array,
    B_wqkv: jax.Array,
    B_wo: jax.Array,
    gate_w: jax.Array,
):
    xT = A_x.reshape(S, D).T
    gw = gate_w.reshape(1, D)

    full = lambda shape: pl.BlockSpec(shape, lambda i: (0,) * len(shape))
    outT = pl.pallas_call(
        _kernel,
        grid=(NQ,),
        in_specs=[full((D, S)), full((D, 3 * D)), full((D, 3 * D)), full((D, D)),
                  full((D, D)), full((1, D))],
        out_specs=pl.BlockSpec((D, BQ), lambda i: (0, i)),
        out_shape=jax.ShapeDtypeStruct((D, S), jnp.bfloat16),
        scratch_shapes=[
            pltpu.VMEM((NG, S, 128), jnp.bfloat16),
            pltpu.VMEM((NG, 128, S), jnp.bfloat16),
            pltpu.VMEM((NH, HP, S), jnp.bfloat16),
            pltpu.VMEM((D, 2 * DP), jnp.bfloat16),
            pltpu.VMEM((8, S), jnp.float32),
            pltpu.VMEM((NH, HP, BQ), jnp.bfloat16),
            pltpu.VMEM((S, BQ), jnp.float32),
            pltpu.VMEM((S, BQ), jnp.float32),
            pltpu.VMEM((8, BQ), jnp.float32),
        ],
        compiler_params=pltpu.CompilerParams(
            dimension_semantics=("arbitrary",),
            vmem_limit_bytes=100 * 1024 * 1024),
    )(xT, A_wqkv, B_wqkv, A_wo, B_wo, gw)
    return outT.T.reshape(1, S, D)
```

```python
import math

import jax
import jax.numpy as jnp
import jax.experimental.pallas as pl
import jax.experimental.pallas.tpu as pltpu

S = 2048
D = 448
H = 16
DH = 28
HP = 32
DP = H * HP
NH = 2 * H
NG = NH // 4
SQ = 512
SUB = S // SQ
CK = 128
NC = S // CK
TC = 1024
QSCALE = (DH ** -0.5) * math.log2(math.e)


def _kernel(xT_hbm, wa_hbm, wb_hbm, woa_hbm, wob_hbm, gw_hbm, o_hbm,
            xT_ref, wa_ref, wb_ref, woa_ref, wob_ref, gw_ref, ob_ref,
            sems, xsems, osems,
            wk_scr, wqT_scr, wvT_scr, woT_scr,
            k_scr, qT_scr, vT_scr, g_scr, oT_scr, sa_scr, sb_scr, m_scr):
    copies = [pltpu.make_async_copy(src, dst, sems.at[i]) for i, (src, dst) in enumerate((
        (gw_hbm, gw_ref), (wa_hbm, wa_ref), (wb_hbm, wb_ref),
        (woa_hbm, woa_ref), (wob_hbm, wob_ref)))]

    def x_copy(t):
        t0 = pl.multiple_of(t * TC, TC)
        return pltpu.make_async_copy(xT_hbm.at[:, pl.ds(t0, TC)], xT_ref.at[:, pl.ds(t0, TC)],
                                     xsems.at[t])

    def o_copy(u):
        c0 = pl.multiple_of(u * SQ, SQ)
        return pltpu.make_async_copy(ob_ref.at[:, pl.ds(c0, SQ)], o_hbm.at[:, pl.ds(c0, SQ)],
                                     osems.at[u])

    copies[1].start()
    copies[0].start()
    x_copy(0).start()
    copies[2].start()
    for t in range(1, S // TC):
        x_copy(t).start()
    copies[3].start()
    copies[4].start()
    for mod, w_ref in enumerate((wa_ref, wb_ref)):
        copies[1 + mod].wait()
        parts = []
        for h in range(H):
            parts.append(w_ref[:, D + DH * h:D + DH * (h + 1)])
            parts.append(jnp.zeros((D, HP - DH), jnp.bfloat16))
        wk_scr[mod] = jnp.concatenate(parts, axis=1)
        wqT_scr[mod] = w_ref[:, 0:D].T
        wvT_scr[mod] = w_ref[:, 2 * D:3 * D].T
    copies[0].wait()
    gw = jnp.broadcast_to(gw_ref[...], (8, D))

    def proj(t, carry):
        t0 = pl.multiple_of(t * TC, TC)
        x_copy(t).wait()
        xT = xT_ref[:, pl.ds(t0, TC)]
        x = xT.T
        zpad = jnp.zeros((HP - DH, TC), jnp.float32)
        rows = jax.lax.broadcasted_iota(jnp.int32, (HP - DH, TC), 0)
        opad = jnp.where(rows == 0, 1.0, 0.0).astype(jnp.float32)
        for mod in range(2):
            kf = jnp.dot(x, wk_scr[mod], preferred_element_type=jnp.float32)
            for j in range(4):
                k_scr[4 * mod + j, pl.ds(t0, TC), :] = kf[:, 128 * j:128 * (j + 1)].astype(jnp.bfloat16)
            qf = jnp.dot(wqT_scr[mod], xT, preferred_element_type=jnp.float32) * QSCALE
            for h in range(H):
                blk = jnp.concatenate([qf[DH * h:DH * (h + 1), :], zpad], axis=0)
                qT_scr[4 * mod + h // 4, HP * (h % 4):HP * (h % 4 + 1), pl.ds(t0, TC)] = (
                    blk.astype(jnp.bfloat16))
            vf = jnp.dot(wvT_scr[mod], xT, preferred_element_type=jnp.float32)
            for h in range(H):
                blk = jnp.concatenate([vf[DH * h:DH * (h + 1), :], opad], axis=0)
                vT_scr[H * mod + h, :, pl.ds(t0, TC)] = blk.astype(jnp.bfloat16)
        gl = jnp.dot(gw, xT, preferred_element_type=jnp.float32)
        g_scr[:, pl.ds(t0, TC)] = jax.nn.sigmoid(gl)
        return carry

    jax.lax.fori_loop(0, S // TC, proj, 0)

    for mod, wo_ref in enumerate((woa_ref, wob_ref)):
        copies[3 + mod].wait()
        parts = []
        for h in range(H):
            parts.append(wo_ref[DH * h:DH * (h + 1), :])
            parts.append(jnp.zeros((HP - DH, D), jnp.bfloat16))
        woT_scr[:, DP * mod:DP * (mod + 1)] = jnp.concatenate(parts, axis=0).T

    def qmask(hn, u):
        qT = qT_scr[hn // 4, :, u * SQ:(u + 1) * SQ]
        rows = jax.lax.broadcasted_iota(jnp.int32, (128, SQ), 0)
        return jnp.where((rows // HP) == hn % 4, qT, jnp.zeros_like(qT))

    def qk_chunk(hn, qm, c, u, s_nxt, m_part):
        s = jnp.dot(k_scr[hn // 4, c * CK:(c + 1) * CK, :], qm,
                    preferred_element_type=jnp.float32)
        s_nxt[c * CK:(c + 1) * CK, u * SQ:(u + 1) * SQ] = s
        mx = jnp.max(s.reshape(CK // 8, 8, SQ), axis=0)
        return mx if m_part is None else jnp.maximum(m_part, mx)

    def store_max(u, m_part):
        m_scr[:, u * SQ:(u + 1) * SQ] = jnp.broadcast_to(
            jnp.max(m_part, axis=0, keepdims=True), (8, SQ))

    def finish(h, cols, acc):
        l = acc[DH:DH + 1, :]
        g = g_scr[0:1, cols]
        gate = jnp.where(h < H, g, 1.0 - g)
        oT_scr[h, :, cols] = (acc * (gate / l)).astype(jnp.bfloat16)

    for u in range(SUB):
        qm0 = qmask(0, u)
        mp = None
        for c in range(NC):
            mp = qk_chunk(0, qm0, c, u, sa_scr, mp)
        store_max(u, mp)

    def stage(h, s_cur, s_nxt):
        for u in range(SUB):
            cols = slice(u * SQ, (u + 1) * SQ)
            m_cur = m_scr[0:1, cols]
            qm = qmask(h + 1, u)
            m_part = None
            acc = None
            for c in range(NC):
                if c < NC - 1:
                    m_part = qk_chunk(h + 1, qm, c, u, s_nxt, m_part)
                p = jnp.exp2(s_cur[c * CK:(c + 1) * CK, cols] - m_cur).astype(jnp.bfloat16)
                d = jnp.dot(vT_scr[h, :, c * CK:(c + 1) * CK], p,
                            preferred_element_type=jnp.float32)
                acc = d if acc is None else acc + d
            m_part = qk_chunk(h + 1, qm, NC - 1, u, s_nxt, m_part)
            finish(h, cols, acc)
            store_max(u, m_part)

    def body(h, carry):
        @pl.when(h % 2 == 0)
        def _():
            stage(h, sa_scr, sb_scr)

        @pl.when(h % 2 == 1)
        def _():
            stage(h, sb_scr, sa_scr)
        return carry

    jax.lax.fori_loop(0, NH - 1, body, 0)

    def tail(u, carry):
        cols = pl.ds(pl.multiple_of(u * SQ, SQ), SQ)
        m_cur = m_scr[0:1, cols]
        acc = None
        oacc = None
        for c in range(NC):
            p = jnp.exp2(sb_scr[c * CK:(c + 1) * CK, cols] - m_cur).astype(jnp.bfloat16)
            d = jnp.dot(vT_scr[NH - 1, :, c * CK:(c + 1) * CK], p,
                        preferred_element_type=jnp.float32)
            acc = d if acc is None else acc + d
            j = c // 2
            if c % 2 == 1 and j < NG - 1:
                oj = oT_scr[4 * j:4 * (j + 1), :, cols].reshape(128, SQ)
                e = jnp.dot(woT_scr[:, 128 * j:128 * (j + 1)], oj,
                            preferred_element_type=jnp.float32)
                oacc = e if oacc is None else oacc + e
        finish(NH - 1, cols, acc)
        oj = oT_scr[NH - 4:NH, :, cols].reshape(128, SQ)
        oacc = oacc + jnp.dot(woT_scr[:, 128 * (NG - 1):128 * NG], oj,
                              preferred_element_type=jnp.float32)
        ob_ref[:, cols] = oacc.astype(ob_ref.dtype)
        o_copy(u).start()
        return carry

    jax.lax.fori_loop(0, SUB, tail, 0)
    for u in range(SUB):
        o_copy(u).wait()


@jax.jit
def pallas_gated_mix__mha_block__softmax_full_mha__prompt_kernel(
    A_x: jax.Array,
    A_wqkv: jax.Array,
    A_wo: jax.Array,
    B_x: jax.Array,
    B_wqkv: jax.Array,
    B_wo: jax.Array,
    gate_w: jax.Array,
):
    xT = A_x.reshape(S, D).T
    gw = gate_w.reshape(1, D)

    outT = pl.pallas_call(
        _kernel,
        in_specs=[pl.BlockSpec(memory_space=pl.ANY)] * 6,
        out_specs=pl.BlockSpec(memory_space=pl.ANY),
        out_shape=jax.ShapeDtypeStruct((D, S), jnp.bfloat16),
        scratch_shapes=[
            pltpu.VMEM((D, S), jnp.bfloat16),
            pltpu.VMEM((D, 3 * D), jnp.bfloat16),
            pltpu.VMEM((D, 3 * D), jnp.bfloat16),
            pltpu.VMEM((D, D), jnp.bfloat16),
            pltpu.VMEM((D, D), jnp.bfloat16),
            pltpu.VMEM((1, D), jnp.bfloat16),
            pltpu.VMEM((D, S), jnp.bfloat16),
            pltpu.SemaphoreType.DMA((5,)),
            pltpu.SemaphoreType.DMA((S // TC,)),
            pltpu.SemaphoreType.DMA((SUB,)),
            pltpu.VMEM((2, D, DP), jnp.bfloat16),
            pltpu.VMEM((2, D, D), jnp.bfloat16),
            pltpu.VMEM((2, D, D), jnp.bfloat16),
            pltpu.VMEM((D, 2 * DP), jnp.bfloat16),
            pltpu.VMEM((NG, S, 128), jnp.bfloat16),
            pltpu.VMEM((NG, 128, S), jnp.bfloat16),
            pltpu.VMEM((NH, HP, S), jnp.bfloat16),
            pltpu.VMEM((8, S), jnp.float32),
            pltpu.VMEM((NH, HP, S), jnp.bfloat16),
            pltpu.VMEM((S, S), jnp.float32),
            pltpu.VMEM((S, S), jnp.float32),
            pltpu.VMEM((8, S), jnp.float32),
        ],
        compiler_params=pltpu.CompilerParams(vmem_limit_bytes=110 * 1024 * 1024),
    )(xT, A_wqkv, B_wqkv, A_wo, B_wo, gw)
    return outT.T.reshape(1, S, D)
```
